```python
import os as _os
_os.environ.setdefault('JAX_PLATFORMS', 'cpu')
import jax
import jax.numpy as jnp

def _softmax(x, axis=-1):
    return jax.nn.softmax(x, axis=axis)

def _gelu(x):
    return jax.nn.gelu(x, approximate=True)

def _silu(x):
    return jax.nn.silu(x)

def _sigmoid(x):
    return jax.nn.sigmoid(x)

def _layernorm(x, axis=-1, eps=1e-05):
    m = jnp.mean(x, axis=axis, keepdims=True)
    v = jnp.var(x, axis=axis, keepdims=True)
    return (x - m) / jnp.sqrt(v + eps)

def _scatter_add(tgt, idx, src, axis=0):
    return tgt.at[idx].add(src)

def _segment_sum(src, seg, n):
    return jax.ops.segment_sum(src, seg, n)

class _Rng:

    def __init__(self, key):
        self._k = key

    def _next(self):
        self._k, sub = jax.random.split(self._k)
        return sub

    def normal(self, shape):
        return jax.random.normal(self._next(), shape, dtype=jnp.bfloat16)

    def randint(self, lo, hi, shape):
        return jax.random.randint(self._next(), shape, lo, hi, dtype=jnp.int32)

    def uniform(self, shape, lo=0.0, hi=1.0):
        return jax.random.uniform(self._next(), shape, jnp.bfloat16, lo, hi)

    def permutation(self, n):
        return jax.random.permutation(self._next(), n)
kernel_name = 'sequential_preLN__linear_attn_block__mixer_gmlp__prompt'

def setup_inputs():
    _rng = _Rng(jax.random.key(int.from_bytes(__import__("os").urandom(4), "little")))
    _w = lambda a: (lambda t: t.astype(jnp.bfloat16) if jnp.issubdtype(t.dtype, jnp.floating) else t)(jnp.asarray(a))

    def _A_setup():
        B, S, D = (1, 2048, 512)
        return {'x': _w((lambda *s: _rng.normal(s) * 0.05)(B, S, D)), 'wqkv': _w((lambda *s: _rng.normal(s) * 0.05)(D, 3 * D)), 'wo': _w((lambda *s: _rng.normal(s) * 0.05)(D, D))}
    _A_in = _A_setup()

    def _B_setup():
        B, S, D, F = (1, 2048, 512, 1792)
        Fh = F // 2
        return {'x': _w((lambda *s: _rng.normal(s) * 0.05)(B, S, D)), 'w_in': _w((lambda *s: _rng.normal(s) * 0.4)(D, 2 * Fh)), 'w_sp': _w(0.01 * (lambda *s: _rng.normal(s) * 0.4)(S, S)), 'b_sp': _w(1.0 + 0.01 * (lambda *s: _rng.normal(s) * 0.05)(S)), 'w_out': _w((lambda *s: _rng.normal(s) * 0.05)(Fh, D))}
    _B_in = _B_setup()
    return {'A_x': _A_in['x'], 'A_wqkv': _A_in['wqkv'], 'A_wo': _A_in['wo'], 'B_x': _B_in['x'], 'B_w_in': _B_in['w_in'], 'B_w_sp': _B_in['w_sp'], 'B_b_sp': _B_in['b_sp'], 'B_w_out': _B_in['w_out']}

def reference(A_x, A_wqkv, A_wo, B_x, B_w_in, B_w_sp, B_b_sp, B_w_out):

    def _A_ref(x, wqkv, wo):
        B, S, D = x.shape
        H = 32
        Dh = D // H
        qkv = (lambda x, *d: x.transpose(*d))((x @ wqkv).reshape(B, S, 3, H, Dh), 2, 0, 3, 1, 4)
        q, k, v = (qkv[0], qkv[1], qkv[2])
        phi = lambda t: jnp.where(t > 0, t + 1, jnp.exp(t)) + 1e-06
        pq, pk = (phi(q), phi(k))
        kv = jnp.einsum('bhsd,bhse->bhde', pk, v)
        z = jnp.einsum('bhsd->bhd', pk)
        num = jnp.einsum('bhqd,bhde->bhqe', pq, kv)
        den = jnp.einsum('bhqd,bhd->bhq', pq, z)[..., None] + 1e-06
        o = num / den
        return (lambda x, *d: x.transpose(*d))(o, 0, 2, 1, 3).reshape(B, S, D) @ wo

    def _B_ref(x, w_in, w_sp, b_sp, w_out):
        B, S, D = x.shape
        F = w_in.shape[-1]
        Fh = F // 2
        z = _gelu(jnp.einsum('bsd,df->bsf', x, w_in))
        z1 = z[..., :Fh].copy()
        z2 = _layernorm(z[..., Fh:], axis=-1)
        g = jnp.einsum('ts,bsf->btf', w_sp, z2) + b_sp[None, :, None]
        return jnp.einsum('bsf,fd->bsd', z1 * g, w_out)
    x = A_x
    h = x + _A_ref(_layernorm(x, axis=-1), A_wqkv, A_wo)
    h2 = h + _B_ref(_layernorm(h, axis=-1), B_w_in, B_w_sp, B_b_sp, B_w_out)
    return h2
```

```python
import functools
import math
import jax
import jax.numpy as jnp
import numpy as np
from jax import lax
import jax.experimental.pallas as pl
import jax.experimental.pallas.tpu as pltpu

S, D, H, DH, FH = 2048, 512, 32, 16, 896
F32, BF16 = jnp.float32, jnp.bfloat16
C1 = math.sqrt(2.0 / math.pi)
C2 = C1 * 0.044715
NF = FH // 128


def _rows(i, T, off=0, n=None):
    n = T if n is None else n
    if isinstance(i, int):
        return pl.ds(i * T + off, n)
    return pl.ds(pl.multiple_of(i * T + off, n), n)


def _loop(lo, hi, body, unroll=False):
    if hi - lo <= 0:
        return
    if unroll or hi - lo == 1:
        for i in range(lo, hi):
            body(i)
    else:
        def f(i, c):
            body(i)
            return c
        lax.fori_loop(lo, hi, f, 0)


def _interleave(main, fill):
    n, m = len(main), len(fill)
    k = 0
    for a, f in enumerate(main):
        f()
        tgt = ((a + 1) * m + n - 1) // n
        while k < min(tgt, m):
            fill[k]()
            k += 1
    while k < m:
        fill[k]()
        k += 1


def make(newton=True, T=256, T3=256, vmem_mb=100, RC=32, unroll1=False, unroll2=False, **cp):
    N = S // T
    N3 = S // T3

    def kernel(x_hbm, wqkv_hbm, wo_hbm, win_hbm, wsp_hbm, bsp_ref, wout_hbm, o_hbm,
               x_v, wqkv_v, wo_v, win_v, wsp_v, wout_v, xn_v, pq_v, kv_v, zs_v, m_v, h_v, hn_v, z2_v, o_v, b_v,
               sx, sw, so, sq):
        def xcp(i):
            r = _rows(i, T)
            return pltpu.make_async_copy(x_hbm.at[r], x_v.at[r], sx.at[i])
        def ocp(i):
            r = _rows(i, T3)
            return pltpu.make_async_copy(o_v.at[r], o_hbm.at[r], so.at[i])
        def wcp(c):
            cs = pl.ds(c * 512, 512)
            return pltpu.make_async_copy(wqkv_hbm.at[:, cs], wqkv_v.at[:, cs], sq.at[c])
        wo_cp = pltpu.make_async_copy(wo_hbm, wo_v, sw.at[2])
        win_cp = pltpu.make_async_copy(win_hbm, win_v, sw.at[3])
        wout_cp = pltpu.make_async_copy(wout_hbm, wout_v, sw.at[4])
        wsp_cp = pltpu.make_async_copy(wsp_hbm, wsp_v, sw.at[5])

        xcp(0).start()
        wcp(1).start(priority=1)
        wcp(2).start(priority=1)
        wcp(0).start(priority=1)

        brow = bsp_ref[...].astype(F32)
        for i in range(S // 128):
            blk = jnp.broadcast_to(brow[i:i + 1, :], (128, 128))
            b_v[pl.ds(i * 128, 128), :] = blk.T
        zs_v[...] = jnp.zeros_like(zs_v)
        kv_v[...] = jnp.zeros_like(kv_v)

        def lnx_chunks(i):
            def chunk(c):
                def f():
                    r = _rows(i, T, c * RC, RC)
                    x = x_v[r, :].astype(F32)
                    xc = x - jnp.mean(x, axis=-1, keepdims=True)
                    var = jnp.mean(xc * xc, axis=-1, keepdims=True)
                    xn_v[r, :] = (xc * lax.rsqrt(var + 1e-5)).astype(BF16)
                return f
            return [chunk(c) for c in range(T // RC)]

        def qkv_items(i):
            r = _rows(i, T)
            xn = xn_v[r, :]
            st = {}
            def kdot(j):
                def f():
                    k = jnp.dot(xn, wqkv_v[:, D + 128 * j:D + 128 * (j + 1)], preferred_element_type=F32)
                    pk = jnp.where(k > 0, k + 1.0, jnp.exp(k)) + 1e-6
                    zs_v[:, 128 * j:128 * (j + 1)] += jnp.sum(pk.reshape(T // 8, 8, 128), axis=0)
                    st['k', j] = pk.astype(BF16)
                return f
            def vdot(j):
                def f():
                    v = jnp.dot(xn, wqkv_v[:, 2 * D + 128 * j:2 * D + 128 * (j + 1)], preferred_element_type=F32)
                    st['v', j] = v.astype(BF16)
                return f
            def kvdot(j):
                def f():
                    kv_v[j] += lax.dot_general(st['k', j], st['v', j], (((0,), (0,)), ((), ())), preferred_element_type=F32)
                return f
            def qdot(j):
                def f():
                    q = jnp.dot(xn, wqkv_v[:, 128 * j:128 * (j + 1)], preferred_element_type=F32)
                    pq_v[r, 128 * j:128 * (j + 1)] = jnp.where(q > 0, q + 1.0, jnp.exp(q)) + 1e-6
                return f
            return [kdot(0), vdot(0), kdot(1), vdot(1), kvdot(0), kdot(2), vdot(2), kvdot(1), kdot(3), vdot(3), kvdot(2),
                    qdot(0), kvdot(3), qdot(1), qdot(2), qdot(3)]

        xcp(0).wait()
        xcp(1).start(priority=1)
        for f in lnx_chunks(0):
            f()
        a = qkv_items(0)
        wcp(1).wait()
        for i in range(2, N):
            xcp(i).start(priority=1)
        for t in (0, 2, 5, 8):
            a[t]()
        wcp(2).wait()
        wo_cp.start(priority=1)
        win_cp.start(priority=1)
        for t in (1, 3, 4, 6, 7, 9, 10):
            a[t]()
        wcp(0).wait()
        xcp(1).wait()
        wout_cp.start(priority=1)
        wsp_cp.start(priority=1)
        _interleave(a[11:], lnx_chunks(1))

        def p1(i):
            xcp(i + 1).wait()
            _interleave(qkv_items(i), lnx_chunks(i + 1))
        _loop(1, N - 1, p1, unroll1)
        for f in qkv_items(N - 1):
            f()

        wo_cp.wait()
        ri = lax.broadcasted_iota(jnp.int32, (128, 128), 0) // DH
        ci = lax.broadcasted_iota(jnp.int32, (128, 128), 1) // DH
        bd = ri == ci
        for j in range(4):
            sl = slice(j * 128, (j + 1) * 128)
            kvbd = jnp.where(bd, kv_v[j], 0.0).astype(BF16)
            m_v[sl, :] = jnp.dot(kvbd, wo_v[sl, :], preferred_element_type=F32).astype(BF16)
        zrow = jnp.sum(zs_v[...], axis=0, keepdims=True)
        ones_bd = jnp.where(bd, 1.0, 0.0).astype(BF16)

        def den_items(i):
            r = _rows(i, T)
            st = {}
            def den(j):
                def f():
                    sl = slice(j * 128, (j + 1) * 128)
                    pq = pq_v[r, sl]
                    t = (pq * zrow[:, sl]).astype(BF16)
                    dn = jnp.dot(t, ones_bd, preferred_element_type=F32) + 1e-6
                    rc = pltpu.reciprocal(dn, approx=True)
                    if newton:
                        rc = rc * (2.0 - dn * rc)
                    st[j] = (pq * rc).astype(BF16)
                return f
            return [den(j) for j in range(4)], st

        def att_items(i, st):
            r = _rows(i, T)
            def att(j):
                def f():
                    sl = slice(j * 128, (j + 1) * 128)
                    p = jnp.concatenate([st[a] for a in range(4)], axis=1)
                    h_v[r, sl] = x_v[r, sl].astype(F32) + jnp.dot(p, m_v[:, sl], preferred_element_type=F32)
                return f
            return [att(j) for j in range(4)]

        def lnh_chunks(i):
            def chunk(c):
                def f():
                    r = _rows(i, T, c * RC, RC)
                    h = h_v[r, :]
                    hc = h - jnp.mean(h, axis=-1, keepdims=True)
                    var = jnp.mean(hc * hc, axis=-1, keepdims=True)
                    hn_v[r, :] = (hc * lax.rsqrt(var + 1e-5)).astype(BF16)
                return f
            return [chunk(c) for c in range(T // RC)]

        def up2_items(i):
            r = _rows(i, T)
            hn = hn_v[r, :]
            st = {}
            def up(j):
                def f():
                    u = jnp.dot(hn, win_v[:, FH + 128 * j:FH + 128 * (j + 1)], preferred_element_type=F32)
                    hu = 0.5 * u
                    st[j] = hu + hu * jnp.tanh(u * (C1 + C2 * (u * u)))
                return f
            def lnz(c):
                def f():
                    rc = _rows(i, T, c * RC, RC)
                    z = jnp.concatenate([st[a][c * RC:(c + 1) * RC] for a in range(NF)], axis=1)
                    zc = z - jnp.mean(z, axis=-1, keepdims=True)
                    var = jnp.mean(zc * zc, axis=-1, keepdims=True)
                    z2_v[rc, :] = (zc * lax.rsqrt(var + 1e-5)).astype(BF16)
                return f
            return [up(j) for j in range(NF)], [lnz(c) for c in range(T // RC)]

        def z1_items(i):
            r = _rows(i, T3)
            hn = hn_v[r, :]
            st = {}
            def up(j):
                def f():
                    u = jnp.dot(hn, win_v[:, 128 * j:128 * (j + 1)], preferred_element_type=F32)
                    hu = 0.5 * u
                    st[j] = hu + hu * jnp.tanh(u * (C1 + C2 * (u * u)))
                return f
            return [up(j) for j in range(NF)], st

        def out_items(i, st):
            r = _rows(i, T3)
            def f():
                g = jnp.dot(wsp_v[r, :], z2_v[...], preferred_element_type=F32)
                b = b_v[r, :]
                g = g + jnp.concatenate([b] * NF, axis=1)
                z1 = jnp.concatenate([st[a] for a in range(NF)], axis=1)
                y = (z1 * g).astype(BF16)
                o = h_v[r, :] + jnp.dot(y, wout_v[...], preferred_element_type=F32)
                o_v[r, :] = o.astype(BF16)
                ocp(i).start()
            return [f]

        def run(items):
            for f in items:
                f()

        d0, s0 = den_items(0)
        run(d0)
        d1, s1 = den_items(1)
        run(d1)
        run(att_items(0, s0))
        win_cp.wait()
        _interleave(att_items(1, s1), lnh_chunks(0))

        def p2(s):
            ups, lnz = up2_items(s)
            dn, sd = den_items(s + 2)
            _interleave(ups[:2] + dn + ups[2:], lnh_chunks(s + 1))
            _interleave(att_items(s + 2, sd), lnz)
        _loop(0, N - 2, p2, unroll2)
        ups, lnz6 = up2_items(N - 2)
        _interleave(ups, lnh_chunks(N - 1))
        ups, lnz7 = up2_items(N - 1)
        _interleave(ups, lnz6)
        wout_cp.wait()
        wsp_cp.wait()
        z1i, z1s = z1_items(0)
        _interleave(z1i, lnz7)
        run(out_items(0, z1s))

        def p3(i):
            a, st = z1_items(i)
            run(a)
            run(out_items(i, st))
        _loop(1, N3, p3)
        for i in range(N3):
            ocp(i).wait()

    @jax.jit
    def fn(A_x, A_wqkv, A_wo, B_x, B_w_in, B_w_sp, B_b_sp, B_w_out):
        any_spec = pl.BlockSpec(memory_space=pl.ANY)
        out = pl.pallas_call(
            kernel,
            out_shape=jax.ShapeDtypeStruct((S, D), BF16),
            in_specs=[any_spec, any_spec, any_spec, any_spec, any_spec,
                      pl.BlockSpec(memory_space=pltpu.VMEM), any_spec],
            out_specs=any_spec,
            scratch_shapes=[
                pltpu.VMEM((S, D), BF16), pltpu.VMEM((D, 3 * D), BF16), pltpu.VMEM((D, D), BF16),
                pltpu.VMEM((D, 2 * FH), BF16), pltpu.VMEM((S, S), BF16), pltpu.VMEM((FH, D), BF16),
                pltpu.VMEM((S, D), BF16), pltpu.VMEM((S, D), F32), pltpu.VMEM((4, 128, 128), F32),
                pltpu.VMEM((8, D), F32),
                pltpu.VMEM((D, D), BF16), pltpu.VMEM((S, D), F32), pltpu.VMEM((S, D), BF16),
                pltpu.VMEM((S, FH), BF16), pltpu.VMEM((S, D), BF16), pltpu.VMEM((S, 128), F32),
                pltpu.SemaphoreType.DMA((N,)), pltpu.SemaphoreType.DMA((6,)),
                pltpu.SemaphoreType.DMA((N3,)), pltpu.SemaphoreType.DMA((3,)),
            ],
            compiler_params=pltpu.CompilerParams(vmem_limit_bytes=vmem_mb * 1024 * 1024, **cp),
        )(A_x.reshape(S, D), A_wqkv, A_wo, B_w_in, B_w_sp, B_b_sp.reshape(S // 128, 128), B_w_out)
        return out.reshape(1, S, D)
    return fn


_FN = make(flags={'XLA_TPU_EVENLY_DISTRIBUTE_CRITICAL_NODES': True})


def pallas_sequential_preLN__linear_attn_block__mixer_gmlp__prompt_kernel(
        A_x, A_wqkv, A_wo, B_x, B_w_in, B_w_sp, B_b_sp, B_w_out):
    return _FN(A_x, A_wqkv, A_wo, B_x, B_w_in, B_w_sp, B_b_sp, B_w_out)
```

```python
import math

import jax
import jax.numpy as jnp
from jax import lax
import jax.experimental.pallas as pl
import jax.experimental.pallas.tpu as pltpu

S, D, DH, FH = 2048, 512, 16, 896
F32, BF16 = jnp.float32, jnp.bfloat16
C1 = math.sqrt(2.0 / math.pi)
C2 = C1 * 0.044715
NF = FH // 128
B = 256
NB = S // B
RC = 32
KSP = 128
OSPLIT = 4
DPOS = 3


def _rows(i, off=0, n=B):
    if isinstance(i, int):
        return pl.ds(i * B + off, n)
    return pl.ds(pl.multiple_of(i * B + off, RC), n)


def _loop(lo, hi, step, body, unroll=1):
    def f(it, c):
        for u in range(unroll):
            body(lo + (it * unroll + u) * step)
        return c
    lax.fori_loop(0, (hi - lo) // (step * unroll), f, 0)


def _run(items):
    for f in items:
        f()


def _interleave(main, fill):
    n, m = len(main), len(fill)
    k = 0
    for a, f in enumerate(main):
        f()
        while k < ((a + 1) * m + n - 1) // n:
            fill[k]()
            k += 1


def _dot(a, b):
    return jnp.dot(a, b, preferred_element_type=F32)


def _ln(x):
    xc = x - jnp.mean(x, axis=-1, keepdims=True)
    var = jnp.mean(xc * xc, axis=-1, keepdims=True)
    return xc * lax.rsqrt(var + 1e-5)


def _phi(t):
    return jnp.where(t > 0, t + 1.0, jnp.exp(t)) + 1e-6


def _gelu(u):
    hu = 0.5 * u
    return hu + hu * jnp.tanh(u * (C1 + C2 * (u * u)))


def _kernel(x_hbm, wqkv_hbm, wo_hbm, win_hbm, wsp_hbm, bsp_hbm, wout_hbm, o_hbm,
            x_v, wqkv_v, wo_v, win_v, wsp_v, wout_v, bsp_v,
            xn_v, pq_v, g_v, zs_v, m_v, h_v, hn_v, z2_v, o_v, b_v,
            sx, sw, so, sq):
    def xcp(i):
        r = _rows(i)
        return pltpu.make_async_copy(x_hbm.at[r], x_v.at[r], sx.at[i])

    def ocp(i, off, n, k):
        r = _rows(i, off, n)
        return pltpu.make_async_copy(o_v.at[r], o_hbm.at[r], so.at[i + k * NB])

    def wcp(c):
        c0, n = ((0, D), (D, KSP), (2 * D, D), (D + KSP, D - KSP))[c]
        cs = pl.ds(c0, n)
        return pltpu.make_async_copy(wqkv_hbm.at[:, cs], wqkv_v.at[:, cs], sq.at[c])

    wo_cp = pltpu.make_async_copy(wo_hbm, wo_v, sw.at[0])
    win_cp = pltpu.make_async_copy(win_hbm, win_v, sw.at[1])
    wout_cp = pltpu.make_async_copy(wout_hbm, wout_v, sw.at[2])
    wsp_cp = pltpu.make_async_copy(wsp_hbm, wsp_v, sw.at[3])
    bsp_cp = pltpu.make_async_copy(bsp_hbm, bsp_v, sw.at[4])

    xcp(0).start()
    wcp(1).start(priority=1)
    wcp(3).start(priority=1)
    wcp(0).start(priority=1)

    zs_v[...] = jnp.zeros_like(zs_v)
    g_v[...] = jnp.zeros_like(g_v)

    def ln_chunks(src, dst, i, m=1):
        def chunk(c):
            def f():
                r = _rows(i, c * RC, RC)
                dst[r, :] = _ln(src[r, :].astype(F32)).astype(BF16)
            return f
        return [chunk(c) for c in range(m * B // RC)]

    def qkg_items(i, m=1):
        r = _rows(i, 0, m * B)
        xn = xn_v[r, :]
        st = {}

        def kdot(j):
            def f():
                pk = _phi(_dot(xn, wqkv_v[:, D + 128 * j:D + 128 * (j + 1)]))
                zs_v[:, 128 * j:128 * (j + 1)] += jnp.sum(pk.reshape(m * B // 8, 8, 128), axis=0)
                st[j] = pk.astype(BF16).T
            return f

        def gdot(j, w):
            def f():
                if 'T' not in st:
                    st['T'] = jnp.concatenate([st[a] for a in range(4)], axis=0)
                g_v[:, w * j:w * (j + 1)] += _dot(st['T'], xn[:, w * j:w * (j + 1)])
            return f

        def qdot(j):
            def f():
                q = _dot(xn, wqkv_v[:, 128 * j:128 * (j + 1)])
                pq_v[r, 128 * j:128 * (j + 1)] = _phi(q).astype(BF16)
            return f

        gw = 128 if m > 1 else 256
        return ([kdot(j) for j in range(4)], [qdot(j) for j in range(4)],
                [gdot(j, gw) for j in range(D // gw)])

    def qkg_all(i, m=1):
        ks, qs, gs = qkg_items(i, m)
        return ks + qs + gs

    xcp(0).wait()
    xcp(1).start(priority=1)
    _run(ln_chunks(x_v, xn_v, 0))
    ks, qs, gs = qkg_items(0)
    wcp(1).wait()
    for i in range(2, NB):
        xcp(i).start(priority=1)
    _run(ks[:KSP // 128])
    wcp(3).wait()
    _run(ks[KSP // 128:])
    _run(gs)
    wcp(0).wait()
    xcp(1).wait()
    xcp(2).wait()
    wcp(2).start(priority=1)
    wo_cp.start(priority=1)
    win_cp.start(priority=1)
    bsp_cp.start(priority=1)
    _interleave(qs, ln_chunks(x_v, xn_v, 1, 2))

    def p1(i):
        xcp(i + 2).wait()
        nx = jnp.minimum(i + 3, NB - 1)

        @pl.when(i + 3 < NB)
        def _():
            xcp(nx).wait()

        _interleave(qkg_all(i, 2), ln_chunks(x_v, xn_v, i + 2) + ln_chunks(x_v, xn_v, nx))

    _loop(1, NB - 1, 2, p1)
    wo_cp.wait()
    wcp(2).wait()
    bsp_cp.wait()
    win_cp.wait()
    wout_cp.start(priority=1)
    wsp_cp.start(priority=1)
    _run(qkg_all(NB - 1))

    brow = bsp_v[...].astype(F32)
    for i in range(S // 128):
        b_v[pl.ds(i * 128, 128), :] = jnp.broadcast_to(brow[i:i + 1, :], (128, 128)).T

    ri = lax.broadcasted_iota(jnp.int32, (128, 128), 0) // DH
    ci = lax.broadcasted_iota(jnp.int32, (128, 128), 1) // DH
    bd = ri == ci
    for j in range(4):
        sl = slice(j * 128, (j + 1) * 128)
        kv = _dot(g_v[sl, :].astype(BF16), wqkv_v[:, 2 * D + j * 128:2 * D + (j + 1) * 128])
        m_v[sl, :] = _dot(jnp.where(bd, kv, 0.0).astype(BF16), wo_v[sl, :]).astype(BF16)
    zrow = jnp.sum(zs_v[...], axis=0, keepdims=True)
    zbd = [jnp.where(bd, jnp.broadcast_to(zrow[:, j * 128:(j + 1) * 128], (128, 128)).T, 0.0).astype(BF16)
           for j in range(4)]

    def den_items(i):
        r = _rows(i)
        st = {}

        def den(j):
            def f():
                pq = pq_v[r, j * 128:(j + 1) * 128]
                dn = _dot(pq, zbd[j]) + 1e-6
                st[j] = (pq.astype(F32) * pltpu.reciprocal(dn, approx=True)).astype(BF16)
            return f
        return [den(j) for j in range(4)], st

    def att_items(i, st):
        r = _rows(i)

        def att(j):
            def f():
                sl = slice(j * 128, (j + 1) * 128)
                p = jnp.concatenate([st[a] for a in range(4)], axis=1)
                h_v[r, sl] = x_v[r, sl].astype(F32) + _dot(p, m_v[:, sl])
            return f
        return [att(j) for j in range(4)]

    def gelu_items(i, m, col0):
        hn = hn_v[_rows(i, 0, m * B), :]
        st = {}

        def up(j):
            def f():
                st[j] = _gelu(_dot(hn, win_v[:, col0 + 128 * j:col0 + 128 * (j + 1)]))
            return f
        return [up(j) for j in range(NF)], st

    def up2_items(i):
        ups, st = gelu_items(i, 1, FH)

        def lnz(c):
            def f():
                z = jnp.concatenate([st[a][c * RC:(c + 1) * RC] for a in range(NF)], axis=1)
                z2_v[_rows(i, c * RC, RC), :] = _ln(z).astype(BF16)
            return f
        return ups, [lnz(c) for c in range(B // RC)]

    d0, s0 = den_items(0)
    _run(d0)
    d1, s1 = den_items(1)
    _run(d1)
    _run(att_items(0, s0))
    _interleave(att_items(1, s1), ln_chunks(h_v, hn_v, 0))

    def p2(s):
        ups, lnz = up2_items(s)
        dn, sd = den_items(s + 2)
        _interleave(ups[:DPOS] + dn + ups[DPOS:], ln_chunks(h_v, hn_v, s + 1))
        _interleave(att_items(s + 2, sd), lnz)

    _loop(0, NB - 2, 1, p2, unroll=2)
    wout_cp.wait()
    wsp_cp.wait()
    ups, lnz6 = up2_items(NB - 2)
    _interleave(ups, ln_chunks(h_v, hn_v, NB - 1))
    ups, lnz7 = up2_items(NB - 1)
    _interleave(ups, lnz6)

    n_out = 2 * B // OSPLIT

    def p3_items(i, lead):
        r = _rows(i, 0, 2 * B)
        z1, st = gelu_items(i, 2, 0)

        def gate(j):
            def f():
                g = _dot(wsp_v[r, :], z2_v[:, 128 * j:128 * (j + 1)])
                st['y', j] = (st[j] * (g + b_v[r, :])).astype(BF16)
            return f

        def fin():
            y = jnp.concatenate([st['y', a] for a in range(NF)], axis=1)
            for k in range(OSPLIT):
                rk = _rows(i, k * n_out, n_out)
                o = h_v[rk, :] + _dot(y[k * n_out:(k + 1) * n_out], wout_v[...])
                o_v[rk, :] = o.astype(BF16)
                ocp(i, k * n_out, n_out, k).start()

        seq = []
        for j in range(NF):
            if j >= lead:
                seq.append(z1[j])
            seq.append(gate(j))
        return z1[:lead], seq + [fin]

    head, rest = p3_items(0, 2)
    _interleave(head, lnz7)
    _run(rest)

    def p3(i):
        head, rest = p3_items(i, 1)
        _run(head)
        _run(rest)

    _loop(2, NB, 2, p3)
    for i in range(0, NB, 2):
        for k in range(OSPLIT):
            ocp(i, k * n_out, n_out, k).wait()


@jax.jit
def pallas_sequential_preLN__linear_attn_block__mixer_gmlp__prompt_kernel(
        A_x, A_wqkv, A_wo, B_x, B_w_in, B_w_sp, B_b_sp, B_w_out):
    hbm = pl.BlockSpec(memory_space=pl.ANY)
    out = pl.pallas_call(
        _kernel,
        out_shape=jax.ShapeDtypeStruct((S, D), BF16),
        in_specs=[hbm] * 7,
        out_specs=hbm,
        scratch_shapes=[
            pltpu.VMEM((S, D), BF16),
            pltpu.VMEM((D, 3 * D), BF16),
            pltpu.VMEM((D, D), BF16),
            pltpu.VMEM((D, 2 * FH), BF16),
            pltpu.VMEM((S, S), BF16),
            pltpu.VMEM((FH, D), BF16),
            pltpu.VMEM((S // 128, 128), BF16),
            pltpu.VMEM((S, D), BF16),
            pltpu.VMEM((S, D), BF16),
            pltpu.VMEM((D, D), F32),
            pltpu.VMEM((8, D), F32),
            pltpu.VMEM((D, D), BF16),
            pltpu.VMEM((S, D), F32),
            pltpu.VMEM((S, D), BF16),
            pltpu.VMEM((S, FH), BF16),
            pltpu.VMEM((S, D), BF16),
            pltpu.VMEM((S, 128), F32),
            pltpu.SemaphoreType.DMA((NB,)),
            pltpu.SemaphoreType.DMA((5,)),
            pltpu.SemaphoreType.DMA((OSPLIT * NB,)),
            pltpu.SemaphoreType.DMA((4,)),
        ],
        compiler_params=pltpu.CompilerParams(
            vmem_limit_bytes=100 * 1024 * 1024,
            flags={"XLA_TPU_EVENLY_DISTRIBUTE_CRITICAL_NODES": True},
        ),
    )(A_x.reshape(S, D), A_wqkv, A_wo, B_w_in, B_w_sp, B_b_sp.reshape(S // 128, 128), B_w_out)
    return out.reshape(1, S, D)
```
